```python
import jax
import jax.numpy as jnp

def _softmax(x, axis=-1):
    return jax.nn.softmax(x, axis=axis)
def _gelu(x):
    return jax.nn.gelu(x, approximate=True)
def _silu(x):
    return jax.nn.silu(x)
def _sigmoid(x):
    return jax.nn.sigmoid(x)
def _layernorm(x, axis=-1, eps=1e-5):
    m = jnp.mean(x, axis=axis, keepdims=True)
    v = jnp.var(x, axis=axis, keepdims=True)
    return (x - m) / jnp.sqrt(v + eps)
def _scatter_add(tgt, idx, src, axis=0):
    return tgt.at[idx].add(src)
def _segment_sum(src, seg, n):
    return jax.ops.segment_sum(src, seg, n)
class _Rng:
    def __init__(self, key):
        self._k = key
    def _next(self):
        self._k, sub = jax.random.split(self._k)
        return sub
    def normal(self, shape):
        return jax.random.normal(self._next(), shape, dtype=jnp.bfloat16)
    def randint(self, lo, hi, shape):
        return jax.random.randint(self._next(), shape, lo, hi, dtype=jnp.int32)
    def uniform(self, shape, lo=0.0, hi=1.0):
        return jax.random.uniform(self._next(), shape, jnp.bfloat16, lo, hi)
    def permutation(self, n):
        return jax.random.permutation(self._next(), n)


kernel_name = 'standalone__gqa_block_cached__near_ridge'

def _fwd_setup_inputs():
    _rng = _Rng(jax.random.key(int.from_bytes(__import__("os").urandom(4), "little")))
    _w = (lambda a: (lambda t: t.astype(jnp.bfloat16) if jnp.issubdtype(t.dtype, jnp.floating) else t)(jnp.asarray(a)))
    B, Sq, D = 16, 64, 640
    Hq, Hkv, Sk, Dh = 32, 32, 512, 192
    assert Hq % Hkv == 0, (Hq, Hkv)
    return {
        "x": _w((lambda *s: _rng.normal(s) * 0.05)(B, Sq, D)),
        "k_cache": _w((lambda *s: _rng.normal(s) * 0.05)(B, Hkv, Sk, Dh)),
        "v_cache": _w((lambda *s: _rng.normal(s) * 0.05)(B, Hkv, Sk, Dh)),
        "wq": _w((lambda *s: _rng.normal(s) * 0.05)(D, Hq * Dh) * (D ** -0.5)),
        "wo": _w((lambda *s: _rng.normal(s) * 0.05)(Hq * Dh, D) * ((Hq * Dh) ** -0.5)),
    }

def _fwd_reference(x, k_cache, v_cache, wq, wo):
    B, Sq, D = x.shape
    Hq, Dh = 32, 192
    Hkv = k_cache.shape[1]
    rep = Hq // Hkv
    q = (lambda x, *d: x.transpose(*d))((x @ wq).reshape(B, Sq, Hq, Dh), 0, 2, 1, 3)
    k = jnp.repeat(k_cache, rep, axis=1)
    v = jnp.repeat(v_cache, rep, axis=1)
    scores = jnp.einsum("bhqd,bhkd->bhqk", q, k) * (Dh ** -0.5)
    p = _softmax(scores, axis=-1)
    o = jnp.einsum("bhqk,bhkd->bhqd", p, v)
    return (lambda x, *d: x.transpose(*d))(o, 0, 2, 1, 3).reshape(B, Sq, Hq * Dh) @ wo


def setup_inputs():
    _inp = _fwd_setup_inputs()
    _gk = jax.random.fold_in(jax.random.key(int.from_bytes(__import__("os").urandom(4), "little")), 2**31 - 1)
    _shapes = [[16, 64, 640]]
    _dtypes = ['bfloat16']
    _gks = jax.random.split(_gk, len(_shapes))
    _gs = [jax.random.normal(k, s, dtype=jnp.dtype(d)) * 0.05 for k, s, d in zip(_gks, _shapes, _dtypes)]
    _inp["grad_out"] = _gs[0]
    return _inp

def reference(x, k_cache, v_cache, wq, wo, grad_out):
    _const = dict()
    def _f(*_d):
        return _fwd_reference(**{'x': _d[0], 'k_cache': _d[1], 'v_cache': _d[2], 'wq': _d[3], 'wo': _d[4], **_const})
    _out, _vjp = jax.vjp(_f, x, k_cache, v_cache, wq, wo)
    _grads = _vjp(grad_out)
    _out0 = jnp.asarray(_out)
    return (_out0, *[jnp.asarray(_g) for _g in _grads])
```

```python
import jax
import jax.numpy as jnp
from jax import lax
from jax.experimental import pallas as pl
from jax.experimental.pallas import tpu as pltpu

B, SQ, D = 16, 64, 640
H, SK, DH = 32, 512, 192
M = B * SQ
NP = H // 2
PW = 2 * DH
F32 = jnp.float32
BF16 = jnp.bfloat16
SCALE = DH ** -0.5


def nn(a, b):
    return lax.dot_general(a, b, (((1,), (0,)), ((), ())), preferred_element_type=F32)


def nt(a, b):
    return lax.dot_general(a, b, (((1,), (1,)), ((), ())), preferred_element_type=F32)


def make(do_dma=True, do_compute=True, NB=4, rtail=64, wtail=1, n_pre=4, n_def=3, flags=None, scopes=False,
         wb=8, wr=32, nobc=True):
    NJ = B // NB
    RB = NB * SQ
    NT = NP * NJ
    HALF = NJ // 2

    def kern(x_hbm, g_hbm, kt_hbm, vt_hbm, wq_hbm, wo_hbm,
             out_hbm, dx_hbm, dkt_hbm, dvt_hbm, dwq_hbm, dwo_hbm,
             xb, gb, xt, kb, vb, dkb, dvb, wqb, wob, dwqb, dwob,
             wqacc, woacc, oacc, dxacc, ob16, dxb16,
             sem_x, sem_0, sem_r, sem_o, sem_f):
        def col(p):
            return p * PW if isinstance(p, int) else pl.multiple_of(p * PW, 128)

        def rows(j):
            return pl.ds(j * RB if isinstance(j, int) else pl.multiple_of(j * RB, RB), RB)

        def wq_copy(p, sem):
            return pltpu.make_async_copy(wq_hbm.at[:, pl.ds(col(p), PW)], wqb.at[p % 2], sem)

        def wo_copy(p, n, sem):
            return pltpu.make_async_copy(wo_hbm.at[pl.ds(col(p), n * PW)], wob.at[pl.ds(col(p), n * PW)], sem)

        def first_copies(j):
            bs = pl.ds(j * NB, NB)
            return [pltpu.make_async_copy(kt_hbm.at[bs, pl.ds(0, PW)], kb.at[0, bs], sem_0.at[0, j]),
                    pltpu.make_async_copy(vt_hbm.at[bs, pl.ds(0, PW)], vb.at[0, bs], sem_0.at[1, j])]

        def xg_copies(j):
            return [pltpu.make_async_copy(x_hbm.at[rows(j)], xb.at[rows(j)], sem_0.at[2, j]),
                    pltpu.make_async_copy(g_hbm.at[rows(j)], gb.at[rows(j)], sem_0.at[3, j])]

        def read_main(p):
            s = p % 2
            lo_b, hi_b = pl.ds(0, B - NB), pl.ds(B - NB, NB)
            n = PW - rtail
            return [wq_copy(p, sem_r.at[0]),
                    pltpu.make_async_copy(kt_hbm.at[:, pl.ds(col(p), PW)], kb.at[s], sem_r.at[1]),
                    pltpu.make_async_copy(vt_hbm.at[lo_b, pl.ds(col(p), PW)], vb.at[s, lo_b], sem_r.at[2]),
                    pltpu.make_async_copy(vt_hbm.at[hi_b, pl.ds(col(p), n)], vb.at[s, hi_b, pl.ds(0, n)], sem_r.at[3])]

        def read_tail(p):
            hi_b = pl.ds(B - NB, NB)
            n = PW - rtail
            return pltpu.make_async_copy(vt_hbm.at[hi_b, pl.ds(col(p) + n, rtail)],
                                         vb.at[p % 2, hi_b, pl.ds(n, rtail)], sem_r.at[4])

        def piece(i, p, b0, nb, r, sem):
            src, dst = ((dkb, dkt_hbm), (dvb, dvt_hbm))[i]
            return pltpu.make_async_copy(src.at[p % 2, pl.ds(b0, nb), pl.ds(r, wr)],
                                         dst.at[pl.ds(b0, nb), pl.ds(col(p) + r, wr)], sem)

        all_pieces = [(i, b0, r) for i in range(2) for b0 in range(0, B, wb) for r in range(0, PW, wr)]
        n_main = len(all_pieces) - wtail

        def write_main(p):
            return [piece(i, p, b0, wb, r, sem_o.at[0]) for i, b0, r in all_pieces[:n_main]]

        def write_tail(p):
            return [piece(i, p, b0, wb, r, sem_o.at[1]) for i, b0, r in all_pieces[n_main:]]

        def dwq_copy(p, sem):
            return pltpu.make_async_copy(dwqb.at[p % 2], dwq_hbm.at[:, pl.ds(col(p), PW)], sem)

        def dwo_copy(p, n, sem):
            return pltpu.make_async_copy(dwob.at[pl.ds(col(p), n * PW)], dwo_hbm.at[pl.ds(col(p), n * PW)], sem)

        def last_copies(j):
            cs = [piece(i, NP - 1, j * NB, NB, r, sem_f.at[0]) for r in range(0, PW, wr) for i in range(2)]
            return cs + [pltpu.make_async_copy(ob16.at[rows(j)], out_hbm.at[rows(j)], sem_f.at[1]),
                         pltpu.make_async_copy(dxb16.at[rows(j)], dx_hbm.at[rows(j)], sem_f.at[2])]

        wq_copy(0, sem_x.at[0]).start()
        wo_copy(0, 1, sem_x.at[1]).start()

        def start_first(j, _):
            for c in xg_copies(j) + first_copies(j):
                c.start()
        lax.fori_loop(0, NJ, start_first, None)
        if do_dma:
            wo_copy(1, 1 + n_pre, sem_r.at[5]).start()
            for c in read_main(1):
                c.start()
            if rtail:
                read_tail(1).start(priority=1)
        oacc[...] = jnp.zeros_like(oacc)
        dxacc[...] = jnp.zeros_like(dxacc)
        wqacc[...] = jnp.zeros_like(wqacc)
        woacc[...] = jnp.zeros_like(woacc)
        wq_copy(0, sem_x.at[0]).wait()
        wo_copy(0, 1, sem_x.at[1]).wait()

        lo = lax.broadcasted_iota(jnp.int32, (SQ, 128), 1) < 64
        lo_t = lax.broadcasted_iota(jnp.int32, (DH, 128), 1) < 64

        def compute(p, j):
            s = p % 2
            rs = rows(j)
            ps_ = pl.ds(col(p), PW)
            g = gb[rs, :]
            q32 = nn(xb[rs, :], wqb[s]) * SCALE
            do32 = nt(g, wob[ps_, :])

            def scores(a32, ref, b):
                mid = a32[:, 128:256]
                am = jnp.concatenate([jnp.where(lo, mid, 0.0), jnp.where(lo, 0.0, mid)], axis=0).astype(BF16)
                s0 = nn(a32[:, 0:128].astype(BF16), ref[s, b, 0:128, :])
                sm = nn(am, ref[s, b, 128:256, :])
                s1 = nn(a32[:, 256:384].astype(BF16), ref[s, b, 256:384, :])
                return s0 + sm[0:SQ], s1 + sm[SQ:]

            def front(u):
                b = j * NB + u
                s01 = scores(q32[u * SQ:(u + 1) * SQ], kb, b)
                dp01 = scores(do32[u * SQ:(u + 1) * SQ], vb, b)
                ps, dss = [], []
                for sc_, dp in zip(s01, dp01):
                    m = jnp.max(sc_, axis=1, keepdims=True)
                    e = jnp.exp(sc_ - m)
                    pr = e * (1.0 / jnp.sum(e, axis=1, keepdims=True))
                    delta = jnp.sum(pr * dp, axis=1, keepdims=True)
                    ps.append(pr.astype(BF16))
                    dss.append((pr * (dp - delta)).astype(BF16))
                return ps, dss

            def back(u, ps, dss):
                b = j * NB + u

                def ctx(w, ref):
                    t0 = nt(w[0], ref[s, b, 0:128, :])
                    tm = nt(jnp.concatenate(w, axis=0), ref[s, b, 128:256, :])
                    t2 = nt(w[1], ref[s, b, 256:384, :])
                    return jnp.concatenate([t0, jnp.where(lo, tm[0:SQ], tm[SQ:]), t2], axis=1)

                rt = jnp.concatenate([q32[u * SQ:(u + 1) * SQ].astype(BF16),
                                      do32[u * SQ:(u + 1) * SQ].astype(BF16)], axis=0).T

                def dkv(h):
                    rth = rt[h * DH:(h + 1) * DH]
                    z = jnp.zeros_like(rth)
                    lhs = jnp.concatenate([jnp.where(lo_t, rth, z), jnp.where(lo_t, z, rth)], axis=0)
                    res = nn(lhs, jnp.concatenate([dss[h], ps[h]], axis=0)).astype(BF16)
                    dkb[s, b, h * DH:(h + 1) * DH, :] = res[0:DH]
                    dvb[s, b, h * DH:(h + 1) * DH, :] = res[DH:]

                o = ctx(ps, vb).astype(BF16)
                dkv(0)
                dq = (ctx(dss, kb) * SCALE).astype(BF16)
                dkv(1)
                return o, dq

            os_, dqs = [], []
            cur = front(0)
            for u in range(NB):
                nxt = front(u + 1) if u + 1 < NB else None
                o, dq = back(u, *cur)
                os_.append(o)
                dqs.append(dq)
                cur = nxt
            o = jnp.concatenate(os_, axis=0)
            dq = jnp.concatenate(dqs, axis=0)
            first = j == 0
            a = nn(o.T, g) + jnp.where(first, 0.0, woacc[...])
            woacc[...] = a
            dwob[ps_, :] = a.astype(BF16)
            a = nn(xt[j], dq) + jnp.where(first, 0.0, wqacc[...])
            wqacc[...] = a
            dwqb[s] = a.astype(BF16)
            oacc[rs, :] += nn(o, wob[ps_, :])
            dxacc[rs, :] += nt(dq, wqb[s])

        def step(t, _):
            p = t // NJ
            j = t % NJ

            @pl.when(p == 0)
            def _():
                for c in xg_copies(j):
                    c.wait()
                xt[j] = xb[rows(j), :].T
                for c in first_copies(j):
                    c.wait()

            if do_dma:
                @pl.when((p > 0) & (j == 0))
                def _():
                    @pl.when(p == 1)
                    def _():
                        wo_copy(1, 1 + n_pre, sem_r.at[5]).wait()

                    @pl.when(p > 1 + n_pre)
                    def _():
                        wo_copy(p, 1, sem_r.at[5]).wait()

                    @pl.when(p > 1)
                    def _():
                        for c in write_tail(p - 2):
                            c.wait()
                    for c in read_main(p):
                        c.wait()
                    dwq_copy(p - 1, sem_o.at[2]).start()

                    @pl.when(p - 1 < NP - 2 - n_def)
                    def _():
                        dwo_copy(p - 1, 1, sem_o.at[3]).start()

                    @pl.when(p == NP - 1)
                    def _():
                        dwo_copy(NP - 2 - n_def, 1 + n_def, sem_o.at[3]).start()
                    for c in write_main(p - 1):
                        c.start()
                    for c in write_tail(p - 1):
                        c.start(priority=1)

                @pl.when((p > 0) & (j == HALF))
                def _():
                    if rtail:
                        read_tail(p).wait()

                    @pl.when(p < NP - 1)
                    def _():
                        dwq_copy(p - 1, sem_o.at[2]).wait()

                        @pl.when(p - 1 < NP - 2 - n_def)
                        def _():
                            dwo_copy(p - 1, 1, sem_o.at[3]).wait()
                        for c in write_main(p - 1):
                            c.wait()
                        @pl.when(p + 1 > 1 + n_pre)
                        def _():
                            wo_copy(p + 1, 1, sem_r.at[5]).start()
                        for c in read_main(p + 1):
                            c.start()
                        if rtail:
                            read_tail(p + 1).start(priority=1)

            if do_compute:
                compute(p, j)

            @pl.when(p == NP - 1)
            def _():
                ob16[rows(j), :] = oacc[rows(j), :].astype(BF16)
                dxb16[rows(j), :] = dxacc[rows(j), :].astype(BF16)
                for c in last_copies(j):
                    c.start()

        lax.fori_loop(0, NT, step, None)
        dwq_copy(NP - 1, sem_x.at[0]).start()
        dwo_copy(NP - 1, 1, sem_x.at[1]).start()
        if do_dma:
            dwq_copy(NP - 2, sem_o.at[2]).wait()
            dwo_copy(NP - 2 - n_def, 1 + n_def, sem_o.at[3]).wait()
            for c in write_main(NP - 2) + write_tail(NP - 2):
                c.wait()
        for j in range(NJ):
            for c in last_copies(j):
                c.wait()
        dwq_copy(NP - 1, sem_x.at[0]).wait()
        dwo_copy(NP - 1, 1, sem_x.at[1]).wait()

    call = pl.pallas_call(
        kern,
        out_shape=[
            jax.ShapeDtypeStruct((M, D), BF16),
            jax.ShapeDtypeStruct((M, D), BF16),
            jax.ShapeDtypeStruct((B, H * DH, SK), BF16),
            jax.ShapeDtypeStruct((B, H * DH, SK), BF16),
            jax.ShapeDtypeStruct((D, H * DH), BF16),
            jax.ShapeDtypeStruct((H * DH, D), BF16),
        ],
        in_specs=[pl.BlockSpec(memory_space=pl.ANY)] * 6,
        out_specs=[pl.BlockSpec(memory_space=pl.ANY)] * 6,
        scratch_shapes=[
            pltpu.VMEM((M, D), BF16), pltpu.VMEM((M, D), BF16),
            pltpu.VMEM((NJ, D, RB), BF16),
            pltpu.VMEM((2, B, PW, SK), BF16), pltpu.VMEM((2, B, PW, SK), BF16),
            pltpu.VMEM((2, B, PW, SK), BF16), pltpu.VMEM((2, B, PW, SK), BF16),
            pltpu.VMEM((2, D, PW), BF16), pltpu.VMEM((H * DH, D), BF16),
            pltpu.VMEM((2, D, PW), BF16), pltpu.VMEM((H * DH, D), BF16),
            pltpu.VMEM((D, PW), F32), pltpu.VMEM((PW, D), F32),
            pltpu.VMEM((M, D), F32), pltpu.VMEM((M, D), F32),
            pltpu.VMEM((M, D), BF16), pltpu.VMEM((M, D), BF16),
            pltpu.SemaphoreType.DMA((2,)), pltpu.SemaphoreType.DMA((4, NJ)),
            pltpu.SemaphoreType.DMA((6,)), pltpu.SemaphoreType.DMA((4,)),
            pltpu.SemaphoreType.DMA((3,)),
        ],
        compiler_params=pltpu.CompilerParams(vmem_limit_bytes=110 * 2 ** 20, flags=flags,
                                             disable_bounds_checks=nobc),
        name="gqa",
    )

    @jax.jit
    def fn(x, k_cache, v_cache, wq, wo, grad_out):
        kt = jnp.transpose(k_cache, (0, 1, 3, 2)).reshape(B, H * DH, SK)
        vt = jnp.transpose(v_cache, (0, 1, 3, 2)).reshape(B, H * DH, SK)
        out, dx, dkt, dvt, dwq, dwo = call(x.reshape(M, D), grad_out.reshape(M, D), kt, vt, wq, wo)
        dk = jnp.transpose(dkt.reshape(B, H, DH, SK), (0, 1, 3, 2))
        dv = jnp.transpose(dvt.reshape(B, H, DH, SK), (0, 1, 3, 2))
        return out.reshape(B, SQ, D), dx.reshape(B, SQ, D), dk, dv, dwq, dwo

    return fn


_fn = make()


@jax.jit
def pallas_standalone__gqa_block_cached__near_ridge_kernel(x, k_cache, v_cache, wq, wo, grad_out):
    return _fn(x, k_cache, v_cache, wq, wo, grad_out)
```

```python
import jax
import jax.numpy as jnp
from jax import lax
from jax.experimental import pallas as pl
from jax.experimental.pallas import tpu as pltpu

B, SQ, D = 16, 64, 640
H, SK, DH = 32, 512, 192
M = B * SQ
PW = 2 * DH
HR = H * DH // 2
ND = HR // PW
NB = 4
NJ = B // NB
RB = NB * SQ
NI = 2 * NJ

WR = 24
NR = PW // WR
GB = 3
B_HEAD = NJ * GB
R_TAIL = 208
W_MAIN = PW - WR

F32 = jnp.float32
BF16 = jnp.bfloat16
SCALE = DH ** -0.5
ALL = slice(None)


def _nn(a, b):
    return lax.dot_general(a, b, (((1,), (0,)), ((), ())), preferred_element_type=F32)


def _nt(a, b):
    return lax.dot_general(a, b, (((1,), (1,)), ((), ())), preferred_element_type=F32)


def _mult(v, n):
    return v if isinstance(v, int) else pl.multiple_of(v, n)


def _loop(lo, hi, body):
    lax.fori_loop(lo, hi, lambda i, _: body(i), None)


def _kernel(x_hbm, g_hbm, kt_hbm, vt_hbm, wq_hbm, wo_hbm,
            out_hbm, dx_hbm, dkt_hbm, dvt_hbm, dwq_hbm, dwo_hbm,
            xb, gb, kb, vb, dkb, dvb, wqb, wob, dwqb, dwob,
            wqacc, woacc, oacc, dxacc, ob, dxb, otb, xtb,
            sem_0, sem_r, sem_w, sem_f):
    copy = pltpu.make_async_copy

    def rows(j):
        return pl.ds(_mult(j * RB, RB), RB)

    def feat(d, off=0, n=PW):
        return pl.ds(_mult(d * PW, 128) + off, n)

    def wcols(d, e):
        return pl.ds(_mult(e * HR + d * PW, 128), PW)

    def wslot(d, e):
        return (1 - e) * (d % 2) + e * (2 + d)

    def first_weights(e):
        return [copy(wq_hbm.at[:, wcols(0, e)], wqb.at[0, e], sem_0.at[0, e]),
                copy(wo_hbm.at[e * ND], wob.at[wslot(0, e)], sem_0.at[1, e])]

    def first_rows(j):
        return [copy(x_hbm.at[rows(j)], xb.at[rows(j)], sem_0.at[2, j]),
                copy(g_hbm.at[rows(j)], gb.at[rows(j)], sem_0.at[3, j])]

    def first_kv(j, e):
        bs = pl.ds(j * NB, NB)
        return [copy(kt_hbm.at[bs, e, feat(0)], kb.at[0, bs, e], sem_0.at[4, 2 * j + e]),
                copy(vt_hbm.at[bs, e, feat(0)], vb.at[0, bs, e], sem_0.at[5, 2 * j + e])]

    def first_group(i, op):
        j = lax.shift_right_logical(i, 1)
        e = i & 1

        @pl.when(j == 0)
        def _():
            for c in first_weights(e):
                op(c)

        @pl.when(e == 0)
        def _():
            for c in first_rows(j):
                op(c)

        for c in first_kv(j, e):
            op(c)

    def upper_wo():
        return copy(wo_hbm.at[pl.ds(ND + 1, ND - 1)], wob.at[pl.ds(wslot(1, 1), ND - 1)], sem_r.at[7])

    def read_main(d):
        s = d % 2
        n = PW - R_TAIL
        lead = pl.ds(0, B - 1)
        return [copy(wq_hbm.at[:, wcols(d, 0)], wqb.at[s, 0], sem_r.at[0]),
                copy(wq_hbm.at[:, wcols(d, 1)], wqb.at[s, 1], sem_r.at[1]),
                copy(wo_hbm.at[d], wob.at[s], sem_r.at[2]),
                copy(kt_hbm.at[:, :, feat(d)], kb.at[s], sem_r.at[3]),
                copy(vt_hbm.at[lead, :, feat(d)], vb.at[s, lead], sem_r.at[4]),
                copy(vt_hbm.at[B - 1, :, feat(d, 0, n)], vb.at[s, B - 1, :, pl.ds(0, n)], sem_r.at[5])]

    def read_tail(d):
        n = PW - R_TAIL
        return copy(vt_hbm.at[B - 1, :, feat(d, n, R_TAIL)], vb.at[d % 2, B - 1, :, pl.ds(n, R_TAIL)],
                    sem_r.at[6])

    def start_reads(d):
        for c in read_main(d):
            c.start()
        read_tail(d).start()

    def dkv_out(i, d, b0, nb, e, r, nr, sem):
        src, dst = ((dkb, dkt_hbm), (dvb, dvt_hbm))[i]
        return copy(src.at[d % 2, pl.ds(b0, nb), e, pl.ds(r, nr)], dst.at[pl.ds(b0, nb), e, feat(d, r, nr)], sem)

    def dwq_out(d, e, sem):
        return copy(dwqb.at[d % 2, e], dwq_hbm.at[:, wcols(d, e)], sem)

    def dwo_out(d, e, n, r, nr, sem):
        return copy(dwob.at[pl.ds(wslot(d, e), n), pl.ds(r, nr)], dwo_hbm.at[pl.ds(e * ND + d, n), pl.ds(r, nr)],
                    sem)

    def rows_out(i, r, nr):
        src, dst = ((ob, out_hbm), (dxb, dx_hbm))[i]
        return copy(src.at[pl.ds(r, nr)], dst.at[pl.ds(r, nr)], sem_f.at[2 + i])

    def start_write_head(d):
        for i in range(2):
            for n in range(NR):
                dkv_out(i, d, B_HEAD, B - B_HEAD, ALL, n * WR, WR, sem_w.at[i]).start()
            dwq_out(d, i, sem_w.at[5 + i]).start()

    def start_write_piece(d, part, i, n):
        last = jnp.where(part == NJ - 1, 1, 0)
        k = 0 if i == 0 else 2 + last * (2 if n * WR >= W_MAIN else 1)
        dkv_out(i, d, part * GB, GB, ALL, n * WR, WR, sem_w.at[k]).start()
        if i == 0 and n % 4 == 1:
            dwo_out(d, 0, 1, pl.multiple_of((part * 4 + n // 4) * WR, 8), WR, sem_w.at[7]).start()

    def wait_write_main(d):
        for e in range(2):
            dwq_out(d, e, sem_w.at[5 + e]).wait()
        dwo_out(d, 0, 1, 0, PW, sem_w.at[7]).wait()
        dkv_out(0, d, 0, B, ALL, 0, PW, sem_w.at[0]).wait()
        dkv_out(1, d, B_HEAD, B - B_HEAD, ALL, 0, PW, sem_w.at[1]).wait()
        dkv_out(1, d, 0, B_HEAD - GB, ALL, 0, PW, sem_w.at[2]).wait()
        dkv_out(1, d, B_HEAD - GB, GB, ALL, 0, W_MAIN, sem_w.at[3]).wait()

    def wait_write_tail(d):
        dkv_out(1, d, B_HEAD - GB, GB, ALL, W_MAIN, PW - W_MAIN, sem_w.at[4]).wait()

    def start_last_slab(u):
        for i in range(2):
            for n in range(NR):
                dkv_out(i, ND - 1, u * GB, GB, ALL, n * WR, WR, sem_f.at[i]).start()

    def start_upper_dwo():
        _loop(0, NR, lambda n: dwo_out(0, 1, ND - 1, pl.multiple_of(n * WR, 8), WR, sem_f.at[8]).start())

    def start_last_rows(h):
        def one(n):
            for i in range(2):
                for j in range(2 * h, 2 * h + 2):
                    rows_out(i, pl.multiple_of(j * RB + n * 32, 32), 32).start()
        _loop(0, RB // 32, one)

    def start_last_chunk(e):
        dwq_out(ND - 1, e, sem_f.at[4 + e]).start()

        def one(n):
            for m in range(2):
                for i in range(2):
                    dkv_out(i, ND - 1, B - NB, NB, e, pl.multiple_of((2 * n + m) * WR, 8), WR, sem_f.at[i]).start()
            dwo_out(ND - 1, e, 1, pl.multiple_of(n * 2 * WR, 16), 2 * WR, sem_f.at[6 + e]).start()
        _loop(0, NR // 2, one)

    def wait_last():
        dwo_out(0, 1, ND - 1, 0, PW, sem_f.at[8]).wait()
        for e in range(2):
            dwq_out(ND - 1, e, sem_f.at[4 + e]).wait()
            dwo_out(ND - 1, e, 1, 0, PW, sem_f.at[6 + e]).wait()
        for i in range(2):
            dkv_out(i, ND - 1, 0, B, ALL, 0, PW, sem_f.at[i]).wait()
        for i in range(2):
            rows_out(i, 0, M).wait()

    def compute(d, j, e):
        s = d % 2
        ws = wslot(d, e)
        rs = rows(j)
        lo = lax.broadcasted_iota(jnp.int32, (SQ, 128), 1) < 64
        lo_t = lax.broadcasted_iota(jnp.int32, (DH, 128), 1) < 64

        def scores(a, ref, b):
            mid = a[:, 128:256]
            am = jnp.concatenate([jnp.where(lo, mid, 0.0), jnp.where(lo, 0.0, mid)], axis=0).astype(BF16)
            s0 = _nn(a[:, 0:128].astype(BF16), ref[s, b, e, 0:128, :])
            sm = _nn(am, ref[s, b, e, 128:256, :])
            s1 = _nn(a[:, 256:384].astype(BF16), ref[s, b, e, 256:384, :])
            return s0 + sm[0:SQ], s1 + sm[SQ:]

        def mix(w, ref, b):
            t0 = _nt(w[0], ref[s, b, e, 0:128, :])
            tm = _nt(jnp.concatenate(w, axis=0), ref[s, b, e, 128:256, :])
            t2 = _nt(w[1], ref[s, b, e, 256:384, :])
            return jnp.concatenate([t0, jnp.where(lo, tm[0:SQ], tm[SQ:]), t2], axis=1)

        def softmax(u):
            prs = []
            for z in scores(q[u * SQ:(u + 1) * SQ], kb, j * NB + u):
                ex = jnp.exp(z - jnp.max(z, axis=1, keepdims=True))
                prs.append(ex * (1.0 / jnp.sum(ex, axis=1, keepdims=True)))
            return prs

        def softmax_grad(u, prs):
            dss = []
            for pr, dp in zip(prs, scores(do[u * SQ:(u + 1) * SQ], vb, j * NB + u)):
                delta = jnp.sum(pr * dp, axis=1, keepdims=True)
                dss.append((pr * (dp - delta)).astype(BF16))
            return [pr.astype(BF16) for pr in prs], dss

        q = _nn(xb[rs, :], wqb[s, e]) * SCALE
        prs = softmax(0)
        do = _nt(gb[rs, :], wob[ws])
        xtb[...] = xb[rs, :].T
        ps, dss = softmax_grad(0, prs)
        o, dq = [], []
        for u in range(NB):
            b = j * NB + u
            rt = jnp.concatenate([q[u * SQ:(u + 1) * SQ].astype(BF16),
                                  do[u * SQ:(u + 1) * SQ].astype(BF16)], axis=0).T
            if u + 1 < NB:
                prs = softmax(u + 1)
            o.append(mix(ps, vb, b).astype(BF16))
            dq.append((mix(dss, kb, b) * SCALE).astype(BF16))
            nxt = softmax_grad(u + 1, prs) if u + 1 < NB else (None, None)
            for h in range(2):
                hs = slice(h * DH, (h + 1) * DH)
                zero = jnp.zeros((DH, 128), BF16)
                lhs = jnp.concatenate([jnp.where(lo_t, rt[hs], zero), jnp.where(lo_t, zero, rt[hs])], axis=0)
                res = _nn(lhs, jnp.concatenate([dss[h], ps[h]], axis=0)).astype(BF16)
                dkb[s, b, e, hs, :] = res[0:DH]
                dvb[s, b, e, hs, :] = res[DH:]
            ps, dss = nxt
        o = jnp.concatenate(o, axis=0)
        dq = jnp.concatenate(dq, axis=0)

        otb[...] = o.T
        acc = _nn(otb[...], gb[rs, :]) + jnp.where(j == 0, 0.0, woacc[e])
        woacc[e] = acc
        dwob[ws] = acc.astype(BF16)
        acc = _nn(xtb[...], dq) + jnp.where(j == 0, 0.0, wqacc[e])
        wqacc[e] = acc
        dwqb[s, e] = acc.astype(BF16)
        acc = oacc[rs, :] + _nn(o, wob[ws])
        oacc[rs, :] = acc
        ob[rs, :] = acc.astype(BF16)
        acc = dxacc[rs, :] + _nt(dq, wqb[s, e])
        dxacc[rs, :] = acc
        dxb[rs, :] = acc.astype(BF16)

    _loop(0, NI, lambda i: first_group(i, lambda c: c.start()))
    upper_wo().start()
    start_reads(1)

    def clear(i):
        r = pl.ds(pl.multiple_of(i * SQ, SQ), SQ)
        oacc[r, :] = jnp.zeros((SQ, D), F32)
        dxacc[r, :] = jnp.zeros((SQ, D), F32)
        for e in range(2):
            wqacc[e, pl.ds(pl.multiple_of(i * (D // B), 8), D // B), :] = jnp.zeros((D // B, PW), F32)
            woacc[e, pl.ds(pl.multiple_of(i * (PW // B), 8), PW // B), :] = jnp.zeros((PW // B, D), F32)
    _loop(0, B, clear)

    def step(t):
        d = lax.shift_right_logical(t, NI.bit_length() - 1)
        i = t & (NI - 1)

        @pl.when((d == 0) | (d == ND - 1) | ((i & (NJ - 1)) == 0))
        def _():
            pl.when(d == 0)(lambda: first_group(i, lambda c: c.wait()))

            @pl.when((d > 0) & (i == 0))
            def _():
                pl.when(d == 1)(lambda: upper_wo().wait())
                pl.when(d > 1)(lambda: wait_write_tail(d - 2))
                for c in read_main(d):
                    c.wait()
                start_write_head(d - 1)

            @pl.when((d > 0) & (i == NJ))
            def _():
                read_tail(d).wait()

                @pl.when(d < ND - 1)
                def _():
                    wait_write_main(d - 1)
                    start_reads(d + 1)

            @pl.when((d == ND - 1) & (i >= NJ))
            def _():
                u = i - NJ
                pl.when(u < NJ - 1)(lambda: _loop(u, jnp.where(u == NJ - 2, NJ, u + 1), start_last_slab))
                pl.when(u == 0)(start_upper_dwo)
                pl.when(u == 1)(lambda: start_last_rows(0))
                pl.when(u == NJ - 1)(lambda: start_last_chunk(0))

        writing = ((d > 0) & (i < NJ), (t >= NI) & ((t & NJ) == 0))
        pieces = [(a, n) for a in range(2) for n in range(NR)]
        for k in range(0, len(pieces), 4):
            @pl.when(writing[k // 4 % 2])
            def _():
                for a, n in pieces[k:k + 4]:
                    start_write_piece(d - 1, i, a, n)

        compute(d, lax.shift_right_logical(i, 1), i & 1)

    _loop(0, ND * NI, step)
    start_last_chunk(1)
    start_last_rows(1)
    wait_write_main(ND - 2)
    wait_write_tail(ND - 2)
    wait_last()


@jax.jit
def pallas_standalone__gqa_block_cached__near_ridge_kernel(
    x: jax.Array,
    k_cache: jax.Array,
    v_cache: jax.Array,
    wq: jax.Array,
    wo: jax.Array,
    grad_out: jax.Array,
):
    assert x.shape == (B, SQ, D) and k_cache.shape == v_cache.shape == (B, H, SK, DH)
    kv = pltpu.VMEM((2, B, 2, PW, SK), BF16)
    out, dx, dkt, dvt, dwq, dwo = pl.pallas_call(
        _kernel,
        out_shape=[
            jax.ShapeDtypeStruct((M, D), BF16),
            jax.ShapeDtypeStruct((M, D), BF16),
            jax.ShapeDtypeStruct((B, 2, HR, SK), BF16),
            jax.ShapeDtypeStruct((B, 2, HR, SK), BF16),
            jax.ShapeDtypeStruct((D, H * DH), BF16),
            jax.ShapeDtypeStruct((2 * ND, PW, D), BF16),
        ],
        in_specs=[pl.BlockSpec(memory_space=pl.ANY)] * 6,
        out_specs=[pl.BlockSpec(memory_space=pl.ANY)] * 6,
        scratch_shapes=[
            pltpu.VMEM((M, D), BF16), pltpu.VMEM((M, D), BF16),
            kv, kv, kv, kv,
            pltpu.VMEM((2, 2, D, PW), BF16), pltpu.VMEM((2 + ND, PW, D), BF16),
            pltpu.VMEM((2, 2, D, PW), BF16), pltpu.VMEM((2 + ND, PW, D), BF16),
            pltpu.VMEM((2, D, PW), F32), pltpu.VMEM((2, PW, D), F32),
            pltpu.VMEM((M, D), F32), pltpu.VMEM((M, D), F32),
            pltpu.VMEM((M, D), BF16), pltpu.VMEM((M, D), BF16),
            pltpu.VMEM((PW, RB), BF16), pltpu.VMEM((D, RB), BF16),
            pltpu.SemaphoreType.DMA((6, NI)), pltpu.SemaphoreType.DMA((8,)),
            pltpu.SemaphoreType.DMA((8,)), pltpu.SemaphoreType.DMA((9,)),
        ],
        compiler_params=pltpu.CompilerParams(vmem_limit_bytes=127 * 2 ** 20, disable_bounds_checks=True),
        name="gqa_block_fwd_bwd",
    )(
        x.reshape(M, D),
        grad_out.reshape(M, D),
        jnp.transpose(k_cache, (0, 1, 3, 2)).reshape(B, 2, HR, SK),
        jnp.transpose(v_cache, (0, 1, 3, 2)).reshape(B, 2, HR, SK),
        wq,
        wo.reshape(2 * ND, PW, D),
    )
    return (
        out.reshape(B, SQ, D),
        dx.reshape(B, SQ, D),
        jnp.transpose(dkt.reshape(B, H, DH, SK), (0, 1, 3, 2)),
        jnp.transpose(dvt.reshape(B, H, DH, SK), (0, 1, 3, 2)),
        dwq,
        dwo.reshape(H * DH, D),
    )
```

```python
import jax
import jax.numpy as jnp
from jax import lax
from jax.experimental import pallas as pl
from jax.experimental.pallas import tpu as pltpu

B, SQ, D = 16, 64, 640
H, SK, DH = 32, 512, 192
M = B * SQ
PW = 2 * DH
HR = H * DH // 2
ND = HR // PW
NB = 4
NJ = B // NB
RB = NB * SQ
NI = 2 * NJ

WR = 24
NR = PW // WR
GB = 3
B_HEAD = NJ * GB
R_TAIL = 208
W_MAIN = PW - WR

F32 = jnp.float32
BF16 = jnp.bfloat16
SCALE = DH ** -0.5
ALL = slice(None)


def _nn(a, b):
    return lax.dot_general(a, b, (((1,), (0,)), ((), ())), preferred_element_type=F32)


def _nt(a, b):
    return lax.dot_general(a, b, (((1,), (1,)), ((), ())), preferred_element_type=F32)


def _mult(v, n):
    return v if isinstance(v, int) else pl.multiple_of(v, n)


def _loop(lo, hi, body):
    lax.fori_loop(lo, hi, lambda i, _: body(i), None)


def _pipeline(x_hbm, g_hbm, kt_hbm, vt_hbm, wq_hbm, wo_hbm,
              out_hbm, dx_hbm, dkt_hbm, dvt_hbm, dwq_hbm, dwo_hbm,
              ob, dxb, sem_out,
              xb, gb, kb, vb, dkb, dvb, wqb, wob, dwqb, dwob,
              wqacc, woacc, oacc, dxacc, otb, xtb,
              sem_0, sem_r, sem_w, sem_f):
    copy = pltpu.make_async_copy

    def rows(j):
        return pl.ds(_mult(j * RB, RB), RB)

    def feat(d, off=0, n=PW):
        return pl.ds(_mult(d * PW, 128) + off, n)

    def wcols(d, e):
        return pl.ds(_mult(e * HR + d * PW, 128), PW)

    def wslot(d, e):
        return (1 - e) * (d % 2) + e * (2 + d)

    def first_weights(e):
        return [copy(wq_hbm.at[:, wcols(0, e)], wqb.at[0, e], sem_0.at[0, e]),
                copy(wo_hbm.at[e * ND], wob.at[wslot(0, e)], sem_0.at[1, e])]

    def first_rows(j):
        return [copy(x_hbm.at[rows(j)], xb.at[rows(j)], sem_0.at[2, j]),
                copy(g_hbm.at[rows(j)], gb.at[rows(j)], sem_0.at[3, j])]

    def first_kv(j, e):
        bs = pl.ds(j * NB, NB)
        return [copy(kt_hbm.at[bs, e, feat(0)], kb.at[0, bs, e], sem_0.at[4, 2 * j + e]),
                copy(vt_hbm.at[bs, e, feat(0)], vb.at[0, bs, e], sem_0.at[5, 2 * j + e])]

    def first_group(i, op):
        j = lax.shift_right_logical(i, 1)
        e = i & 1

        @pl.when(j == 0)
        def _():
            for c in first_weights(e):
                op(c)

        @pl.when(e == 0)
        def _():
            for c in first_rows(j):
                op(c)

        for c in first_kv(j, e):
            op(c)

    def upper_wo():
        return copy(wo_hbm.at[pl.ds(ND + 1, ND - 1)], wob.at[pl.ds(wslot(1, 1), ND - 1)], sem_r.at[7])

    def read_main(d):
        s = d % 2
        n = PW - R_TAIL
        lead = pl.ds(0, B - 1)
        return [copy(wq_hbm.at[:, wcols(d, 0)], wqb.at[s, 0], sem_r.at[0]),
                copy(wq_hbm.at[:, wcols(d, 1)], wqb.at[s, 1], sem_r.at[1]),
                copy(wo_hbm.at[d], wob.at[s], sem_r.at[2]),
                copy(kt_hbm.at[:, :, feat(d)], kb.at[s], sem_r.at[3]),
                copy(vt_hbm.at[lead, :, feat(d)], vb.at[s, lead], sem_r.at[4]),
                copy(vt_hbm.at[B - 1, :, feat(d, 0, n)], vb.at[s, B - 1, :, pl.ds(0, n)], sem_r.at[5])]

    def read_tail(d):
        n = PW - R_TAIL
        return copy(vt_hbm.at[B - 1, :, feat(d, n, R_TAIL)], vb.at[d % 2, B - 1, :, pl.ds(n, R_TAIL)],
                    sem_r.at[6])

    def start_reads(d):
        for c in read_main(d):
            c.start()
        read_tail(d).start()

    def dkv_out(i, d, b0, nb, e, r, nr, sem):
        src, dst = ((dkb, dkt_hbm), (dvb, dvt_hbm))[i]
        return copy(src.at[d % 2, pl.ds(b0, nb), e, pl.ds(r, nr)], dst.at[pl.ds(b0, nb), e, feat(d, r, nr)], sem)

    def dwq_out(d, e, sem):
        return copy(dwqb.at[d % 2, e], dwq_hbm.at[:, wcols(d, e)], sem)

    def dwo_out(d, e, n, r, nr, sem):
        return copy(dwob.at[pl.ds(wslot(d, e), n), pl.ds(r, nr)], dwo_hbm.at[pl.ds(e * ND + d, n), pl.ds(r, nr)],
                    sem)

    def rows_out(i, r, nr):
        src, dst = ((ob, out_hbm), (dxb, dx_hbm))[i]
        return copy(src.at[pl.ds(r, nr)], dst.at[pl.ds(r, nr)], sem_out.at[i])

    def start_write_head(d):
        for i in range(2):
            for n in range(NR):
                dkv_out(i, d, B_HEAD, B - B_HEAD, ALL, n * WR, WR, sem_w.at[i]).start()
            dwq_out(d, i, sem_w.at[5 + i]).start()

    def start_write_piece(d, part, i, n):
        last = jnp.where(part == NJ - 1, 1, 0)
        k = 0 if i == 0 else 2 + last * (2 if n * WR >= W_MAIN else 1)
        dkv_out(i, d, part * GB, GB, ALL, n * WR, WR, sem_w.at[k]).start()
        if i == 0 and n % 4 == 1:
            dwo_out(d, 0, 1, pl.multiple_of((part * 4 + n // 4) * WR, 8), WR, sem_w.at[7]).start()

    def wait_write_main(d):
        for e in range(2):
            dwq_out(d, e, sem_w.at[5 + e]).wait()
        dwo_out(d, 0, 1, 0, PW, sem_w.at[7]).wait()
        dkv_out(0, d, 0, B, ALL, 0, PW, sem_w.at[0]).wait()
        dkv_out(1, d, B_HEAD, B - B_HEAD, ALL, 0, PW, sem_w.at[1]).wait()
        dkv_out(1, d, 0, B_HEAD - GB, ALL, 0, PW, sem_w.at[2]).wait()
        dkv_out(1, d, B_HEAD - GB, GB, ALL, 0, W_MAIN, sem_w.at[3]).wait()

    def wait_write_tail(d):
        dkv_out(1, d, B_HEAD - GB, GB, ALL, W_MAIN, PW - W_MAIN, sem_w.at[4]).wait()

    def start_last_slab(u):
        for i in range(2):
            for n in range(NR):
                dkv_out(i, ND - 1, u * GB, GB, ALL, n * WR, WR, sem_f.at[i]).start()

    def start_upper_dwo():
        _loop(0, NR, lambda n: dwo_out(0, 1, ND - 1, pl.multiple_of(n * WR, 8), WR, sem_f.at[6]).start())

    def start_last_rows(h):
        def one(n):
            for i in range(2):
                for j in range(2 * h, 2 * h + 2):
                    rows_out(i, pl.multiple_of(j * RB + n * 32, 32), 32).start()
        _loop(0, RB // 32, one)

    def start_last_chunk(e):
        dwq_out(ND - 1, e, sem_f.at[2 + e]).start()

        def one(n):
            for m in range(2):
                for i in range(2):
                    dkv_out(i, ND - 1, B - NB, NB, e, pl.multiple_of((2 * n + m) * WR, 8), WR, sem_f.at[i]).start()
            dwo_out(ND - 1, e, 1, pl.multiple_of(n * 2 * WR, 16), 2 * WR, sem_f.at[4 + e]).start()
        _loop(0, NR // 2, one)

    def wait_last():
        dwo_out(0, 1, ND - 1, 0, PW, sem_f.at[6]).wait()
        for e in range(2):
            dwq_out(ND - 1, e, sem_f.at[2 + e]).wait()
            dwo_out(ND - 1, e, 1, 0, PW, sem_f.at[4 + e]).wait()
        for i in range(2):
            dkv_out(i, ND - 1, 0, B, ALL, 0, PW, sem_f.at[i]).wait()

    def compute(d, j, e):
        s = d % 2
        ws = wslot(d, e)
        rs = rows(j)
        lo = lax.broadcasted_iota(jnp.int32, (SQ, 128), 1) < 64
        lo_t = lax.broadcasted_iota(jnp.int32, (DH, 128), 1) < 64

        def scores(a, ref, b):
            mid = a[:, 128:256]
            am = jnp.concatenate([jnp.where(lo, mid, 0.0), jnp.where(lo, 0.0, mid)], axis=0).astype(BF16)
            s0 = _nn(a[:, 0:128].astype(BF16), ref[s, b, e, 0:128, :])
            sm = _nn(am, ref[s, b, e, 128:256, :])
            s1 = _nn(a[:, 256:384].astype(BF16), ref[s, b, e, 256:384, :])
            return s0 + sm[0:SQ], s1 + sm[SQ:]

        def mix(w, ref, b):
            t0 = _nt(w[0], ref[s, b, e, 0:128, :])
            tm = _nt(jnp.concatenate(w, axis=0), ref[s, b, e, 128:256, :])
            t2 = _nt(w[1], ref[s, b, e, 256:384, :])
            return jnp.concatenate([t0, jnp.where(lo, tm[0:SQ], tm[SQ:]), t2], axis=1)

        def softmax(u):
            prs = []
            for z in scores(q[u * SQ:(u + 1) * SQ], kb, j * NB + u):
                ex = jnp.exp(z - jnp.max(z, axis=1, keepdims=True))
                prs.append(ex * (1.0 / jnp.sum(ex, axis=1, keepdims=True)))
            return prs

        def softmax_grad(u, prs):
            dss = []
            for pr, dp in zip(prs, scores(do[u * SQ:(u + 1) * SQ], vb, j * NB + u)):
                delta = jnp.sum(pr * dp, axis=1, keepdims=True)
                dss.append((pr * (dp - delta)).astype(BF16))
            return [pr.astype(BF16) for pr in prs], dss

        q = _nn(xb[rs, :], wqb[s, e]) * SCALE
        prs = softmax(0)
        do = _nt(gb[rs, :], wob[ws])
        xtb[...] = xb[rs, :].T
        ps, dss = softmax_grad(0, prs)
        o, dq = [], []
        for u in range(NB):
            b = j * NB + u
            rt = jnp.concatenate([q[u * SQ:(u + 1) * SQ].astype(BF16),
                                  do[u * SQ:(u + 1) * SQ].astype(BF16)], axis=0).T
            if u + 1 < NB:
                prs = softmax(u + 1)
            o.append(mix(ps, vb, b).astype(BF16))
            dq.append((mix(dss, kb, b) * SCALE).astype(BF16))
            nxt = softmax_grad(u + 1, prs) if u + 1 < NB else (None, None)
            for h in range(2):
                hs = slice(h * DH, (h + 1) * DH)
                zero = jnp.zeros((DH, 128), BF16)
                lhs = jnp.concatenate([jnp.where(lo_t, rt[hs], zero), jnp.where(lo_t, zero, rt[hs])], axis=0)
                res = _nn(lhs, jnp.concatenate([dss[h], ps[h]], axis=0)).astype(BF16)
                dkb[s, b, e, hs, :] = res[0:DH]
                dvb[s, b, e, hs, :] = res[DH:]
            ps, dss = nxt
        o = jnp.concatenate(o, axis=0)
        dq = jnp.concatenate(dq, axis=0)

        otb[...] = o.T
        acc = _nn(otb[...], gb[rs, :]) + jnp.where(j == 0, 0.0, woacc[e])
        woacc[e] = acc
        dwob[ws] = acc.astype(BF16)
        acc = _nn(xtb[...], dq) + jnp.where(j == 0, 0.0, wqacc[e])
        wqacc[e] = acc
        dwqb[s, e] = acc.astype(BF16)
        acc = oacc[rs, :] + _nn(o, wob[ws])
        oacc[rs, :] = acc
        ob[rs, :] = acc.astype(BF16)
        acc = dxacc[rs, :] + _nt(dq, wqb[s, e])
        dxacc[rs, :] = acc
        dxb[rs, :] = acc.astype(BF16)

    _loop(0, NI, lambda i: first_group(i, lambda c: c.start()))
    upper_wo().start()
    start_reads(1)

    def clear(i):
        r = pl.ds(pl.multiple_of(i * SQ, SQ), SQ)
        oacc[r, :] = jnp.zeros((SQ, D), F32)
        dxacc[r, :] = jnp.zeros((SQ, D), F32)
        for e in range(2):
            wqacc[e, pl.ds(pl.multiple_of(i * (D // B), 8), D // B), :] = jnp.zeros((D // B, PW), F32)
            woacc[e, pl.ds(pl.multiple_of(i * (PW // B), 8), PW // B), :] = jnp.zeros((PW // B, D), F32)
    _loop(0, B, clear)

    def step(t):
        d = lax.shift_right_logical(t, NI.bit_length() - 1)
        i = t & (NI - 1)

        @pl.when((d == 0) | (d == ND - 1) | ((i & (NJ - 1)) == 0))
        def _():
            pl.when(d == 0)(lambda: first_group(i, lambda c: c.wait()))

            @pl.when((d > 0) & (i == 0))
            def _():
                pl.when(d == 1)(lambda: upper_wo().wait())
                pl.when(d > 1)(lambda: wait_write_tail(d - 2))
                for c in read_main(d):
                    c.wait()
                start_write_head(d - 1)

            @pl.when((d > 0) & (i == NJ))
            def _():
                read_tail(d).wait()

                @pl.when(d < ND - 1)
                def _():
                    wait_write_main(d - 1)
                    start_reads(d + 1)

            @pl.when((d == ND - 1) & (i >= NJ))
            def _():
                u = i - NJ
                pl.when(u < NJ - 1)(lambda: _loop(u, jnp.where(u == NJ - 2, NJ, u + 1), start_last_slab))
                pl.when(u == 0)(start_upper_dwo)
                pl.when(u == 1)(lambda: start_last_rows(0))
                pl.when(u == NJ - 1)(lambda: start_last_chunk(0))

        writing = ((d > 0) & (i < NJ), (t >= NI) & ((t & NJ) == 0))
        pieces = [(a, n) for a in range(2) for n in range(NR)]
        for k in range(0, len(pieces), 4):
            @pl.when(writing[k // 4 % 2])
            def _():
                for a, n in pieces[k:k + 4]:
                    start_write_piece(d - 1, i, a, n)

        compute(d, lax.shift_right_logical(i, 1), i & 1)

    _loop(0, ND * NI, step)
    start_last_chunk(1)
    start_last_rows(1)
    wait_write_main(ND - 2)
    wait_write_tail(ND - 2)
    wait_last()


def _kernel(*refs):
    out_hbm, dx_hbm = refs[6:8]
    ob, dxb, sem_out = refs[12:15]
    pl.run_scoped(lambda *sems: _pipeline(*refs, *sems),
                  pltpu.SemaphoreType.DMA((6, NI)), pltpu.SemaphoreType.DMA((8,)),
                  pltpu.SemaphoreType.DMA((8,)), pltpu.SemaphoreType.DMA((7,)))
    pltpu.make_async_copy(ob, out_hbm, sem_out.at[0]).wait()
    pltpu.make_async_copy(dxb, dx_hbm, sem_out.at[1]).wait()


@jax.jit
def pallas_standalone__gqa_block_cached__near_ridge_kernel(
    x: jax.Array,
    k_cache: jax.Array,
    v_cache: jax.Array,
    wq: jax.Array,
    wo: jax.Array,
    grad_out: jax.Array,
):
    assert x.shape == (B, SQ, D) and k_cache.shape == v_cache.shape == (B, H, SK, DH)
    kv = pltpu.VMEM((2, B, 2, PW, SK), BF16)
    out, dx, dkt, dvt, dwq, dwo = pl.pallas_call(
        _kernel,
        out_shape=[
            jax.ShapeDtypeStruct((M, D), BF16),
            jax.ShapeDtypeStruct((M, D), BF16),
            jax.ShapeDtypeStruct((B, 2, HR, SK), BF16),
            jax.ShapeDtypeStruct((B, 2, HR, SK), BF16),
            jax.ShapeDtypeStruct((D, H * DH), BF16),
            jax.ShapeDtypeStruct((2 * ND, PW, D), BF16),
        ],
        in_specs=[pl.BlockSpec(memory_space=pl.ANY)] * 6,
        out_specs=[pl.BlockSpec(memory_space=pl.ANY)] * 6,
        scratch_shapes=[
            pltpu.VMEM((M, D), BF16), pltpu.VMEM((M, D), BF16),
            pltpu.SemaphoreType.DMA((2,)),
            pltpu.VMEM((M, D), BF16), pltpu.VMEM((M, D), BF16),
            kv, kv, kv, kv,
            pltpu.VMEM((2, 2, D, PW), BF16), pltpu.VMEM((2 + ND, PW, D), BF16),
            pltpu.VMEM((2, 2, D, PW), BF16), pltpu.VMEM((2 + ND, PW, D), BF16),
            pltpu.VMEM((2, D, PW), F32), pltpu.VMEM((2, PW, D), F32),
            pltpu.VMEM((M, D), F32), pltpu.VMEM((M, D), F32),
            pltpu.VMEM((PW, RB), BF16), pltpu.VMEM((D, RB), BF16),
        ],
        compiler_params=pltpu.CompilerParams(vmem_limit_bytes=127 * 2 ** 20, disable_bounds_checks=True),
        name="gqa_block_fwd_bwd",
    )(
        x.reshape(M, D),
        grad_out.reshape(M, D),
        jnp.transpose(k_cache, (0, 1, 3, 2)).reshape(B, 2, HR, SK),
        jnp.transpose(v_cache, (0, 1, 3, 2)).reshape(B, 2, HR, SK),
        wq,
        wo.reshape(2 * ND, PW, D),
    )
    return (
        out.reshape(B, SQ, D),
        dx.reshape(B, SQ, D),
        jnp.transpose(dkt.reshape(B, H, DH, SK), (0, 1, 3, 2)),
        jnp.transpose(dvt.reshape(B, H, DH, SK), (0, 1, 3, 2)),
        dwq,
        dwo.reshape(H * DH, D),
    )
```
